```python
import jax
import jax.numpy as jnp

def _softmax(x, axis=-1):
    return jax.nn.softmax(x, axis=axis)
def _gelu(x):
    return jax.nn.gelu(x, approximate=True)
def _silu(x):
    return jax.nn.silu(x)
def _sigmoid(x):
    return jax.nn.sigmoid(x)
def _layernorm(x, axis=-1, eps=1e-5):
    m = jnp.mean(x, axis=axis, keepdims=True)
    v = jnp.var(x, axis=axis, keepdims=True)
    return (x - m) / jnp.sqrt(v + eps)
def _scatter_add(tgt, idx, src, axis=0):
    return tgt.at[idx].add(src)
def _segment_sum(src, seg, n):
    return jax.ops.segment_sum(src, seg, n)
class _Rng:
    def __init__(self, key):
        self._k = key
    def _next(self):
        self._k, sub = jax.random.split(self._k)
        return sub
    def normal(self, shape):
        return jax.random.normal(self._next(), shape, dtype=jnp.bfloat16)
    def randint(self, lo, hi, shape):
        return jax.random.randint(self._next(), shape, lo, hi, dtype=jnp.int32)
    def uniform(self, shape, lo=0.0, hi=1.0):
        return jax.random.uniform(self._next(), shape, jnp.bfloat16, lo, hi)
    def permutation(self, n):
        return jax.random.permutation(self._next(), n)


kernel_name = 'standalone__cross_network_dcn_v2__recsys'

def setup_inputs():
    _rng = _Rng(jax.random.key(int.from_bytes(__import__("os").urandom(4), "little")))
    _w = (lambda a: (lambda t: t.astype(jnp.bfloat16) if jnp.issubdtype(t.dtype, jnp.floating) else t)(jnp.asarray(a)))
    B, F, D, L = 16384, 100, 16, 3
    Din = min(F * D, 512)
    R = max(Din // 4, 2)
    sc = Din ** -0.5
    return {
        "x0": _w((lambda *s: _rng.normal(s) * 0.05)(B, Din)),
        "U":  _w((lambda *s: _rng.normal(s) * 0.05)(L, Din, R) * sc),
        "V":  _w((lambda *s: _rng.normal(s) * 0.05)(L, R, Din) * sc),
        "bs": _w((lambda *s: _rng.normal(s) * 0.05)(L, Din)),
    }

def reference(x0, U, V, bs):
    x = x0
    for l in range(U.shape[0]):
        h = jnp.einsum('rd,bd->br', V[l], x)
        h = jnp.einsum('dr,br->bd', U[l], h)
        x = x0 * (h + bs[l]) + x
    return x
```

```python
import jax
import jax.numpy as jnp
from jax import lax
import jax.experimental.pallas as pl
import jax.experimental.pallas.tpu as pltpu

_BM = 1024
_SUB = 256

_NT = (((1,), (1,)), ((), ()))


def _cross_kernel(x0_ref, u_ref, v_ref, b_ref, o_ref):
    num_layers = u_ref.shape[0]
    for s in range(_BM // _SUB):
        rows = pl.ds(s * _SUB, _SUB)
        xb = x0_ref[rows, :]
        x0 = xb.astype(jnp.float32)
        x = x0
        for l in range(num_layers):
            h = lax.dot_general(xb, v_ref[l], _NT, preferred_element_type=jnp.float32)
            h = lax.dot_general(h.astype(jnp.bfloat16), u_ref[l], _NT,
                                preferred_element_type=jnp.float32)
            x = x0 * (h + b_ref[pl.ds(l, 1), :].astype(jnp.float32)) + x
            xb = x.astype(jnp.bfloat16)
        o_ref[rows, :] = xb


@jax.jit
def pallas_standalone__cross_network_dcn_v2__recsys_kernel(
    x0: jax.Array,
    U: jax.Array,
    V: jax.Array,
    bs: jax.Array,
):
    B, D = x0.shape
    L, _, R = U.shape
    return pl.pallas_call(
        _cross_kernel,
        grid=(B // _BM,),
        in_specs=[
            pl.BlockSpec((_BM, D), lambda i: (i, 0)),
            pl.BlockSpec((L, D, R), lambda i: (0, 0, 0)),
            pl.BlockSpec((L, R, D), lambda i: (0, 0, 0)),
            pl.BlockSpec((L, D), lambda i: (0, 0)),
        ],
        out_specs=pl.BlockSpec((_BM, D), lambda i: (i, 0)),
        out_shape=jax.ShapeDtypeStruct((B, D), x0.dtype),
        compiler_params=pltpu.CompilerParams(
            dimension_semantics=("parallel",), vmem_limit_bytes=64 * 1024 * 1024),
    )(x0, U, V, bs)
```

```python
import jax
import jax.numpy as jnp
from jax import lax
import jax.experimental.pallas as pl
import jax.experimental.pallas.tpu as pltpu

_TILE = 256
_HEAD = (1, 2, 5)
_BODY = 14
_TIMER = 64
_LAST = (128, 128)
_ISSUE = ((0, 0, 2), (0, 0, 5), (1, 1, 4))

_NT = (((1,), (1,)), ((), ()))


def _cross_kernel(x_hbm, u_hbm, v_hbm, b_hbm, o_hbm,
                  xbuf, obuf, ubuf, vbuf, bbuf, tbuf, isem, osem, wsem):
    num_rows = xbuf.shape[0]
    num_layers = ubuf.shape[0]
    body_rows = _BODY * _TILE
    starts = [0]
    for n in _HEAD:
        starts.append(starts[-1] + n * _TILE)
    head_rows = starts[-1]
    num_iters = (num_rows - head_rows) // body_rows
    sizes = [n * _TILE for n in _HEAD] + [body_rows]

    def rows(start, size):
        if isinstance(start, int):
            return pl.ds(start, size)
        return pl.ds(pl.multiple_of(start, 16), size)

    def x_copy(start, size, sem):
        r = rows(start, size)
        return pltpu.make_async_copy(x_hbm.at[r, :], xbuf.at[r, :], sem)

    def o_copy(start, size):
        r = rows(start, size)
        return pltpu.make_async_copy(obuf.at[r, :], o_hbm.at[r, :], osem.at[0])

    def w_copies(l):
        return [pltpu.make_async_copy(v_hbm.at[l], vbuf.at[l], wsem.at[l]),
                pltpu.make_async_copy(u_hbm.at[l], ubuf.at[l], wsem.at[l])]

    def seg_copy(i):
        return x_copy(starts[i], sizes[i], isem.at[i % 2])

    def tile(start, hook=None, out_split=None):
        r = rows(start, _TILE)
        for l in range(num_layers):
            src, src_rows = (xbuf, r) if l == 0 else (tbuf.at[l - 1], slice(None))
            if hook is not None:
                hook(2 * l)
            h = lax.dot_general(src[src_rows, :], vbuf[l], _NT,
                                preferred_element_type=jnp.float32)
            if hook is not None:
                hook(2 * l + 1)
            h = lax.dot_general(h.astype(jnp.bfloat16), ubuf[l], _NT,
                                preferred_element_type=jnp.float32)
            bias = bbuf[pl.ds(l, 1), :].astype(jnp.float32)
            x0 = xbuf[r, :].astype(jnp.float32)
            x = x0 if l == 0 else src[src_rows, :].astype(jnp.float32)
            y = (x0 * (h + bias) + x).astype(jnp.bfloat16)
            if l < num_layers - 1:
                tbuf[l] = y
        if out_split is None:
            obuf[r, :] = y
        else:
            p = 0
            for q in out_split:
                obuf[rows(start + p, q), :] = y[p:p + q]
                o_copy(start + p, q).start()
                p += q

    xa = x_copy(0, _TIMER, isem.at[1])
    xb = x_copy(_TIMER, sizes[0] - _TIMER, isem.at[0])
    first = w_copies(0) + [pltpu.make_async_copy(b_hbm, bbuf, wsem.at[0])]
    xa.start()
    xb.start()
    for c in first:
        c.start()
    xa.wait()
    for c in w_copies(1):
        c.start()
    for c in first:
        c.wait()
    xb.wait()

    for i, n in enumerate(_HEAD):
        if i > 0:
            seg_copy(i).wait()
        for j in range(n):
            def hook(k, i=i, j=j):
                if i == 0 and j == 0:
                    if k > 0 and k % 2 == 0:
                        for c in w_copies(k // 2):
                            c.wait()
                    if k % 2 == 0 and k // 2 + 2 < num_layers:
                        for c in w_copies(k // 2 + 2):
                            c.start()
                for t, point in enumerate(_ISSUE):
                    if point == (i, j, k):
                        seg_copy(t + 1).start()
            tile(starts[i] + j * _TILE, hook=hook)

    def body(g, carry):
        base = head_rows + g * body_rows
        slot = (len(_HEAD) + g) % 2
        x_copy(base, body_rows, isem.at[slot]).wait()

        @pl.when(g + 1 < num_iters)
        def _():
            x_copy(base + body_rows, body_rows, isem.at[1 - slot]).start()

        @pl.when(g == 0)
        def _():
            o_copy(0, head_rows).start()

        for j in range(_BODY):
            tile(base + j * _TILE, out_split=_LAST if j == _BODY - 1 else (_TILE,))
        return carry

    lax.fori_loop(0, num_iters, body, None)
    pltpu.make_async_copy(obuf, o_hbm, osem.at[0]).wait()


@jax.jit
def pallas_standalone__cross_network_dcn_v2__recsys_kernel(
    x0: jax.Array,
    U: jax.Array,
    V: jax.Array,
    bs: jax.Array,
):
    B, D = x0.shape
    L = U.shape[0]
    assert L >= 2 and (B - sum(_HEAD) * _TILE) % (_BODY * _TILE) == 0
    any_spec = pl.BlockSpec(memory_space=pl.ANY)
    return pl.pallas_call(
        _cross_kernel,
        in_specs=[any_spec] * 4,
        out_specs=any_spec,
        out_shape=jax.ShapeDtypeStruct((B, D), x0.dtype),
        scratch_shapes=[
            pltpu.VMEM((B, D), x0.dtype),
            pltpu.VMEM((B, D), x0.dtype),
            pltpu.VMEM(U.shape, U.dtype),
            pltpu.VMEM(V.shape, V.dtype),
            pltpu.VMEM(bs.shape, bs.dtype),
            pltpu.VMEM((L - 1, _TILE, D), x0.dtype),
            pltpu.SemaphoreType.DMA((2,)),
            pltpu.SemaphoreType.DMA((1,)),
            pltpu.SemaphoreType.DMA((L,)),
        ],
        compiler_params=pltpu.CompilerParams(
            vmem_limit_bytes=64 * 1024 * 1024, disable_bounds_checks=True),
    )(x0, U, V, bs)
```

```python
import jax
import jax.numpy as jnp
from jax import lax
import jax.experimental.pallas as pl
import jax.experimental.pallas.tpu as pltpu

_TILE = 256
_SEGS = (1, 1, 2, 4, 8, 16)
_LAST_SPLIT = (64, 64, 64, 64)
_ISSUE = ((0, 0, 1), (0, 0, 3), (0, 0, 5), (1, 0, 3), (3, 2, 0))
_OUT_FROM = (5, 0, 0)
_PREFETCH = (5, 4, 0)

_NT = (((1,), (1,)), ((), ()))


def _cross_kernel(x_hbm, u_hbm, v_hbm, b_hbm, o_hbm,
                  xbuf, obuf, ubuf, vbuf, bbuf, tbuf, isem, osem, wsem):
    num_layers = ubuf.shape[0]
    offs = [0]
    for n in _SEGS:
        offs.append(offs[-1] + n * _TILE)
    body_rows = offs[-1]
    num_iters = xbuf.shape[0] // body_rows

    def rows(start, size):
        if isinstance(start, int):
            return pl.ds(start, size)
        return pl.ds(pl.multiple_of(start, 16), size)

    def seg_copy(base, i):
        r = rows(base + offs[i], _SEGS[i] * _TILE)
        return pltpu.make_async_copy(x_hbm.at[r, :], xbuf.at[r, :], isem.at[i])

    def out_copy(start, size):
        r = rows(start, size)
        return pltpu.make_async_copy(obuf.at[r, :], o_hbm.at[r, :], osem.at[0])

    def w_copies(l):
        copies = [pltpu.make_async_copy(v_hbm.at[l], vbuf.at[l], wsem.at[l]),
                  pltpu.make_async_copy(u_hbm.at[l], ubuf.at[l], wsem.at[l])]
        if l == 0:
            copies.append(pltpu.make_async_copy(b_hbm, bbuf, wsem.at[l]))
        return copies

    def start_weights(l):
        for c in w_copies(l):
            c.start()

    def wait_weights(l):
        for c in w_copies(l):
            c.wait()

    def tile(start, hook, out_split):
        r = rows(start, _TILE)
        for l in range(num_layers):
            def load_x():
                return xbuf[r, :] if l == 0 else tbuf[l - 1]

            hook(2 * l)
            h = lax.dot_general(load_x(), vbuf[l], _NT,
                                preferred_element_type=jnp.float32)
            hook(2 * l + 1)
            h = lax.dot_general(h.astype(jnp.bfloat16), ubuf[l], _NT,
                                preferred_element_type=jnp.float32)
            bias = bbuf[pl.ds(l, 1), :].astype(jnp.float32)
            x0 = xbuf[r, :].astype(jnp.float32)
            x = x0 if l == 0 else load_x().astype(jnp.float32)
            y = (x0 * (h + bias) + x).astype(jnp.bfloat16)
            if l < num_layers - 1:
                tbuf[l] = y
        if out_split is None:
            obuf[r, :] = y
        else:
            p = 0
            for q in out_split:
                obuf[rows(start + p, q), :] = y[p:p + q]
                out_copy(start + p, q).start()
                p += q

    seg_copy(0, 0).start()
    start_weights(0)
    start_weights(1)

    def body(g, carry):
        base = g * body_rows
        first = g == 0

        for i, n in enumerate(_SEGS):
            seg_copy(base, i).wait()
            for j in range(n):
                def hook(k, i=i, j=j):
                    if (i, j) == (0, 0) and k % 2 == 0:
                        pl.when(first)(lambda: wait_weights(k // 2))
                        if k // 2 + 2 < num_layers:
                            pl.when(first)(lambda: start_weights(k // 2 + 2))
                    for t, point in enumerate(_ISSUE):
                        if point == (i, j, k):
                            pl.when(first)(lambda: seg_copy(0, t + 1).start())
                    if (i, j, k) == _PREFETCH:
                        @pl.when(g + 1 < num_iters)
                        def _():
                            for t in range(len(_SEGS)):
                                seg_copy(base + body_rows, t).start()
                    if (i, j, k) == _OUT_FROM:
                        out_copy(base, offs[i] + j * _TILE).start()

                if (i, j) < _OUT_FROM[:2]:
                    out_split = None
                elif (i, j) == (len(_SEGS) - 1, n - 1):
                    out_split = _LAST_SPLIT
                else:
                    out_split = (_TILE,)
                tile(base + offs[i] + j * _TILE, hook, out_split)
        return carry

    lax.fori_loop(0, num_iters, body, None)
    pltpu.make_async_copy(obuf, o_hbm, osem.at[0]).wait()


@jax.jit
def pallas_standalone__cross_network_dcn_v2__recsys_kernel(
    x0: jax.Array,
    U: jax.Array,
    V: jax.Array,
    bs: jax.Array,
):
    B, D = x0.shape
    L = U.shape[0]
    assert L == 3 and B % (sum(_SEGS) * _TILE) == 0
    any_spec = pl.BlockSpec(memory_space=pl.ANY)
    return pl.pallas_call(
        _cross_kernel,
        in_specs=[any_spec] * 4,
        out_specs=any_spec,
        out_shape=jax.ShapeDtypeStruct((B, D), x0.dtype),
        scratch_shapes=[
            pltpu.VMEM((B, D), x0.dtype),
            pltpu.VMEM((B, D), x0.dtype),
            pltpu.VMEM(U.shape, U.dtype),
            pltpu.VMEM(V.shape, V.dtype),
            pltpu.VMEM(bs.shape, bs.dtype),
            pltpu.VMEM((L - 1, _TILE, D), x0.dtype),
            pltpu.SemaphoreType.DMA((len(_SEGS),)),
            pltpu.SemaphoreType.DMA((1,)),
            pltpu.SemaphoreType.DMA((L,)),
        ],
        compiler_params=pltpu.CompilerParams(
            vmem_limit_bytes=64 * 1024 * 1024,
            disable_bounds_checks=True,
            flags={"XLA_TPU_RESCHEDULE_DMA_DONES": True},
        ),
    )(x0, U, V, bs)
```

```python
import jax
import jax.numpy as jnp
from jax import lax
import jax.experimental.pallas as pl
import jax.experimental.pallas.tpu as pltpu

_TILE = 256
_SEGS = (1, 1, 2, 4, 8, 16)
_LAST_SPLIT = (64, 64, 64, 64)
_ISSUE = ((0, 0, 1), (0, 0, 3), (0, 0, 5), (1, 0, 3), (3, 2, 0))
_OUT_FROM = (5, 0, 0)
_PREFETCH = (5, 4, 0)

_NT = (((1,), (1,)), ((), ()))


def _cross_kernel(x_hbm, u_hbm, v_hbm, b_hbm, o_hbm,
                  xbuf, obuf, ubuf, vbuf, bbuf, tbuf, isem, osem, wsem):
    num_layers = ubuf.shape[0]
    offs = [0]
    for n in _SEGS:
        offs.append(offs[-1] + n * _TILE)
    body_rows = offs[-1]
    num_iters = xbuf.shape[0] // body_rows

    def rows(start, size):
        if isinstance(start, int):
            return pl.ds(start, size)
        return pl.ds(pl.multiple_of(start, 16), size)

    def seg_copy(base, i):
        r = rows(base + offs[i], _SEGS[i] * _TILE)
        return pltpu.make_async_copy(x_hbm.at[r, :], xbuf.at[r, :], isem.at[i])

    def out_copy(start, size):
        r = rows(start, size)
        return pltpu.make_async_copy(obuf.at[r, :], o_hbm.at[r, :], osem.at[0])

    def w_copies(l):
        sem = isem.at[0] if l == 0 else wsem.at[l - 1]
        return [pltpu.make_async_copy(v_hbm.at[l], vbuf.at[l], sem),
                pltpu.make_async_copy(u_hbm.at[l], ubuf.at[l], sem)]

    def bias_copy():
        return pltpu.make_async_copy(b_hbm, bbuf, isem.at[0])

    def start_weights(l):
        for c in w_copies(l):
            c.start()

    def wait_weights(l):
        for c in w_copies(l):
            c.wait()

    def tile(start, hook, out_split):
        r = rows(start, _TILE)
        for l in range(num_layers):
            def load_x():
                return xbuf[r, :] if l == 0 else tbuf[l - 1]

            hook(2 * l)
            h = lax.dot_general(load_x(), vbuf[l], _NT,
                                preferred_element_type=jnp.float32)
            hook(2 * l + 1)
            h = lax.dot_general(h.astype(jnp.bfloat16), ubuf[l], _NT,
                                preferred_element_type=jnp.float32)
            bias = bbuf[pl.ds(l, 1), :].astype(jnp.float32)
            x0 = xbuf[r, :].astype(jnp.float32)
            x = x0 if l == 0 else load_x().astype(jnp.float32)
            y = (x0 * (h + bias) + x).astype(jnp.bfloat16)
            if l < num_layers - 1:
                tbuf[l] = y
        if out_split is None:
            obuf[r, :] = y
        else:
            p = 0
            for q in out_split:
                obuf[rows(start + p, q), :] = y[p:p + q]
                out_copy(start + p, q).start()
                p += q

    seg_copy(0, 0).start()
    start_weights(0)
    bias_copy().start()
    wait_weights(0)

    def body(g, carry):
        base = g * body_rows
        first = g == 0

        @pl.when(first)
        def _():
            start_weights(1)
            bias_copy().wait()

        for i, n in enumerate(_SEGS):
            seg_copy(base, i).wait()
            for j in range(n):
                def hook(k, i=i, j=j):
                    if (i, j) == (0, 0) and k % 2 == 0:
                        if k > 0:
                            pl.when(first)(lambda: wait_weights(k // 2))
                        if k // 2 + 2 < num_layers:
                            pl.when(first)(lambda: start_weights(k // 2 + 2))
                    for t, point in enumerate(_ISSUE):
                        if point == (i, j, k):
                            pl.when(first)(lambda: seg_copy(0, t + 1).start())
                    if (i, j, k) == _PREFETCH:
                        @pl.when(g + 1 < num_iters)
                        def _():
                            for t in range(len(_SEGS)):
                                seg_copy(base + body_rows, t).start()
                    if (i, j, k) == _OUT_FROM:
                        out_copy(base, offs[i] + j * _TILE).start()

                if (i, j) < _OUT_FROM[:2]:
                    out_split = None
                elif (i, j) == (len(_SEGS) - 1, n - 1):
                    out_split = _LAST_SPLIT
                else:
                    out_split = (_TILE,)
                tile(base + offs[i] + j * _TILE, hook, out_split)
        return carry

    lax.fori_loop(0, num_iters, body, None)
    pltpu.make_async_copy(obuf, o_hbm, osem.at[0]).wait()


@jax.jit
def pallas_standalone__cross_network_dcn_v2__recsys_kernel(
    x0: jax.Array,
    U: jax.Array,
    V: jax.Array,
    bs: jax.Array,
):
    B, D = x0.shape
    L = U.shape[0]
    assert L == 3 and B % (sum(_SEGS) * _TILE) == 0
    any_spec = pl.BlockSpec(memory_space=pl.ANY)
    return pl.pallas_call(
        _cross_kernel,
        in_specs=[any_spec] * 4,
        out_specs=any_spec,
        out_shape=jax.ShapeDtypeStruct((B, D), x0.dtype),
        scratch_shapes=[
            pltpu.VMEM((B, D), x0.dtype),
            pltpu.VMEM((B, D), x0.dtype),
            pltpu.VMEM(U.shape, U.dtype),
            pltpu.VMEM(V.shape, V.dtype),
            pltpu.VMEM(bs.shape, bs.dtype),
            pltpu.VMEM((L - 1, _TILE, D), x0.dtype),
            pltpu.SemaphoreType.DMA((len(_SEGS),)),
            pltpu.SemaphoreType.DMA((1,)),
            pltpu.SemaphoreType.DMA((L - 1,)),
        ],
        compiler_params=pltpu.CompilerParams(
            vmem_limit_bytes=64 * 1024 * 1024,
            disable_bounds_checks=True,
            flags={"XLA_TPU_RESCHEDULE_DMA_DONES": True},
        ),
    )(x0, U, V, bs)
```

```python
import jax
import jax.numpy as jnp
from jax import lax
import jax.experimental.pallas as pl
import jax.experimental.pallas.tpu as pltpu

_TILE = 256
_SEGS = (1, 1, 2, 4, 8, 16)
_LAST_SPLIT = (64, 64, 64, 64)
_ISSUE = ((0, 0, 1), (0, 0, 3), (0, 0, 5), (1, 0, 3), (3, 2, 0))
_OUT_FROM = (5, 0, 0)
_PREFETCH = (5, 4, 0)

_NT = (((1,), (1,)), ((), ()))


def _cross_kernel(x_hbm, u_hbm, v_hbm, b_hbm, o_hbm,
                  xbuf, obuf, ubuf, vbuf, bbuf, tbuf, isem, osem, wsem):
    num_layers = ubuf.shape[0]
    offs = [0]
    for n in _SEGS:
        offs.append(offs[-1] + n * _TILE)
    body_rows = offs[-1]
    num_iters = xbuf.shape[0] // body_rows

    def rows(start, size):
        if isinstance(start, int):
            return pl.ds(start, size)
        return pl.ds(pl.multiple_of(start, 16), size)

    def seg_copy(base, i):
        r = rows(base + offs[i], _SEGS[i] * _TILE)
        return pltpu.make_async_copy(x_hbm.at[r, :], xbuf.at[r, :], isem.at[i])

    def out_copy(start, size):
        r = rows(start, size)
        return pltpu.make_async_copy(obuf.at[r, :], o_hbm.at[r, :], osem.at[0])

    half = ubuf.shape[1] // 2

    def v_copy(l):
        sem = (wsem.at[0], wsem.at[1], wsem.at[0])[l]
        return pltpu.make_async_copy(v_hbm.at[l], vbuf.at[l], sem)

    def u_copy(l, part=None):
        if l == 0:
            r = pl.ds(part * half, half)
            return pltpu.make_async_copy(u_hbm.at[l, r, :], ubuf.at[l, r, :],
                                         wsem.at[2 + part])
        sem = wsem.at[2] if l == 1 else isem.at[0]
        return pltpu.make_async_copy(u_hbm.at[l], ubuf.at[l], sem)

    def bias_copy():
        return pltpu.make_async_copy(b_hbm, bbuf, wsem.at[4])

    def weights_step(k):
        if k == 0:
            u_copy(2).start()
        elif k == 1:
            u_copy(0, 1).wait()
            bias_copy().wait()
        elif k % 2 == 0:
            v_copy(k // 2).wait()
        else:
            u_copy(k // 2).wait()

    def tile(start, hook, out_split):
        r = rows(start, _TILE)
        for l in range(num_layers):
            def load_x():
                return xbuf[r, :] if l == 0 else tbuf[l - 1]

            hook(2 * l)
            h = lax.dot_general(load_x(), vbuf[l], _NT,
                                preferred_element_type=jnp.float32)
            hook(2 * l + 1)
            h = lax.dot_general(h.astype(jnp.bfloat16), ubuf[l], _NT,
                                preferred_element_type=jnp.float32)
            bias = bbuf[pl.ds(l, 1), :].astype(jnp.float32)
            x0 = xbuf[r, :].astype(jnp.float32)
            x = x0 if l == 0 else load_x().astype(jnp.float32)
            y = (x0 * (h + bias) + x).astype(jnp.bfloat16)
            if l < num_layers - 1:
                tbuf[l] = y
        if out_split is None:
            obuf[r, :] = y
        else:
            p = 0
            for q in out_split:
                obuf[rows(start + p, q), :] = y[p:p + q]
                out_copy(start + p, q).start()
                p += q

    seg_copy(0, 0).start()
    v_copy(0).start()
    u_copy(0, 0).start()
    u_copy(0, 1).start()
    bias_copy().start()
    v_copy(1).start()

    def body(g, carry):
        base = g * body_rows
        first = g == 0

        @pl.when(first)
        def _():
            u_copy(0, 0).wait()
            u_copy(1).start()
            v_copy(0).wait()
            v_copy(2).start()

        for i, n in enumerate(_SEGS):
            seg_copy(base, i).wait()
            for j in range(n):
                def hook(k, i=i, j=j):
                    if (i, j) == (0, 0):
                        pl.when(first)(lambda: weights_step(k))
                    for t, point in enumerate(_ISSUE):
                        if point == (i, j, k):
                            pl.when(first)(lambda: seg_copy(0, t + 1).start())
                    if (i, j, k) == _PREFETCH:
                        @pl.when(g + 1 < num_iters)
                        def _():
                            for t in range(len(_SEGS)):
                                seg_copy(base + body_rows, t).start()
                    if (i, j, k) == _OUT_FROM:
                        out_copy(base, offs[i] + j * _TILE).start()

                if (i, j) < _OUT_FROM[:2]:
                    out_split = None
                elif (i, j) == (len(_SEGS) - 1, n - 1):
                    out_split = _LAST_SPLIT
                else:
                    out_split = (_TILE,)
                tile(base + offs[i] + j * _TILE, hook, out_split)
        return carry

    lax.fori_loop(0, num_iters, body, None)
    pltpu.make_async_copy(obuf, o_hbm, osem.at[0]).wait()


@jax.jit
def pallas_standalone__cross_network_dcn_v2__recsys_kernel(
    x0: jax.Array,
    U: jax.Array,
    V: jax.Array,
    bs: jax.Array,
):
    B, D = x0.shape
    L = U.shape[0]
    assert L == 3 and B % (sum(_SEGS) * _TILE) == 0
    any_spec = pl.BlockSpec(memory_space=pl.ANY)
    return pl.pallas_call(
        _cross_kernel,
        in_specs=[any_spec] * 4,
        out_specs=any_spec,
        out_shape=jax.ShapeDtypeStruct((B, D), x0.dtype),
        scratch_shapes=[
            pltpu.VMEM((B, D), x0.dtype),
            pltpu.VMEM((B, D), x0.dtype),
            pltpu.VMEM(U.shape, U.dtype),
            pltpu.VMEM(V.shape, V.dtype),
            pltpu.VMEM(bs.shape, bs.dtype),
            pltpu.VMEM((L - 1, _TILE, D), x0.dtype),
            pltpu.SemaphoreType.DMA((len(_SEGS),)),
            pltpu.SemaphoreType.DMA((1,)),
            pltpu.SemaphoreType.DMA((5,)),
        ],
        compiler_params=pltpu.CompilerParams(
            vmem_limit_bytes=64 * 1024 * 1024,
            disable_bounds_checks=True,
            flags={"XLA_TPU_RESCHEDULE_DMA_DONES": True},
        ),
    )(x0, U, V, bs)
```
